```python
import os as _os
_os.environ.setdefault("JAX_PLATFORMS", "cpu")
import jax
import jax.numpy as jnp

def _softmax(x, axis=-1):
    return jax.nn.softmax(x, axis=axis)
def _gelu(x):
    return jax.nn.gelu(x, approximate=True)
def _silu(x):
    return jax.nn.silu(x)
def _sigmoid(x):
    return jax.nn.sigmoid(x)
def _layernorm(x, axis=-1, eps=1e-5):
    m = jnp.mean(x, axis=axis, keepdims=True)
    v = jnp.var(x, axis=axis, keepdims=True)
    return (x - m) / jnp.sqrt(v + eps)
def _scatter_add(tgt, idx, src, axis=0):
    return tgt.at[idx].add(src)
def _segment_sum(src, seg, n):
    return jax.ops.segment_sum(src, seg, n)
class _Rng:
    def __init__(self, key):
        self._k = key
    def _next(self):
        self._k, sub = jax.random.split(self._k)
        return sub
    def normal(self, shape):
        return jax.random.normal(self._next(), shape, dtype=jnp.bfloat16)
    def randint(self, lo, hi, shape):
        return jax.random.randint(self._next(), shape, lo, hi, dtype=jnp.int32)
    def uniform(self, shape, lo=0.0, hi=1.0):
        return jax.random.uniform(self._next(), shape, jnp.bfloat16, lo, hi)
    def permutation(self, n):
        return jax.random.permutation(self._next(), n)


kernel_name = 'gated_mix__grouped_kv_mqa__glu_gated_reglu__prompt'

def setup_inputs():
    _rng = _Rng(jax.random.key(int.from_bytes(__import__("os").urandom(4), "little")))
    _w = (lambda a: (lambda t: t.astype(jnp.bfloat16) if jnp.issubdtype(t.dtype, jnp.floating) else t)(jnp.asarray(a)))
    def _A_setup():
        B, S, D, H = 1, 2048, 1024, 32
        Dh = D // H
        return {
            "x": _w((lambda *s: _rng.normal(s) * 0.05)(B, S, D)),
            "wq": _w((lambda *s: _rng.normal(s) * 0.2)(D, H * Dh)),
            "wk": _w((lambda *s: _rng.normal(s) * 0.2)(D, Dh)),
            "wv": _w((lambda *s: _rng.normal(s) * 0.05)(D, Dh)),
            "wo": _w((lambda *s: _rng.normal(s) * 0.05)(H * Dh, D)),
        }
    _A_in = _A_setup()

    def _B_setup():
        B, S, D, F = 1, 2048, 1024, 3584
        return {
            "x": _w((lambda *s: _rng.normal(s) * 0.05)(B, S, D)),
            "W_gate": _w((lambda *s: _rng.normal(s) * 0.8)(D, F) * (2.0 / D) ** 0.5),
            "W_up": _w((lambda *s: _rng.normal(s) * 0.8)(D, F) * (2.0 / D) ** 0.5),
            "W_down": _w((lambda *s: _rng.normal(s) * 0.8)(F, D) * (1.0 / F) ** 0.5),
        }
    _B_in = _B_setup()

    return {
        "A_x": _A_in["x"],
        "A_wq": _A_in["wq"],
        "A_wk": _A_in["wk"],
        "A_wv": _A_in["wv"],
        "A_wo": _A_in["wo"],
        "B_x": _B_in["x"],
        "B_W_gate": _B_in["W_gate"],
        "B_W_up": _B_in["W_up"],
        "B_W_down": _B_in["W_down"],
        "gate_w": _w((lambda *s: _rng.normal(s) * 0.05)(1024) * 16.0),
    }

def reference(A_x, A_wq, A_wk, A_wv, A_wo, B_x, B_W_gate, B_W_up, B_W_down, gate_w):
    def _A_ref(x, wq, wk, wv, wo):
        B, S, D = x.shape
        H = 32
        Dh = D // H
        q = (lambda x, *d: x.transpose(*d))((x @ wq).reshape(B, S, H, Dh), 0, 2, 1, 3)
        k = x @ wk
        v = x @ wv
        scores = jnp.einsum("bhqd,bkd->bhqk", q, k) * (Dh ** -0.5)
        p = _softmax(scores, axis=-1)
        o = jnp.einsum("bhqk,bkd->bhqd", p, v)
        return (lambda x, *d: x.transpose(*d))(o, 0, 2, 1, 3).reshape(B, S, H * Dh) @ wo

    def _B_ref(x, W_gate, W_up, W_down):
        gate = jnp.einsum("bsd,df->bsf", x, W_gate)
        up = jnp.einsum("bsd,df->bsf", x, W_up)
        gate = gate * (lambda x, dt: x.astype(dt))(gate > 0, gate.dtype)
        h = gate * up
        return jnp.einsum("bsf,fd->bsd", h, W_down)

    x = A_x
    g = _sigmoid((x * gate_w).sum(-1, keepdims=True))
    a = _A_ref(x, A_wq, A_wk, A_wv, A_wo)
    b = _B_ref(x, B_W_gate, B_W_up, B_W_down)
    return g * a + (1 - g) * b
```

```python
import contextlib
import jax
import jax.numpy as jnp
import numpy as np
from jax import lax
import jax.experimental.pallas as pl
import jax.experimental.pallas.tpu as pltpu

H = 32
LOG2E = float(np.log2(np.e))
NT = (((1,), (1,)), ((), ()))
f32 = jnp.float32
bf16 = jnp.bfloat16
u32 = jnp.uint32


def _dot(a, b):
    return jnp.dot(a, b, preferred_element_type=f32)


LHS = (((0, 1), (3, -1)), ((2, 1), (3, -1)), ((0, 1),), ((3, 1),), ((1, 1), (0, -1)), ((2, 1), (0, -1)), ((1, 1), (3, -1)))
RHS = (((0, 1), (3, -1)), ((0, 1),), ((1, 1), (3, 1)), ((0, 1), (2, 1)), ((3, 1),), ((0, 1), (1, 1)), ((2, 1), (3, 1)))
OUT = (((0, 1), (3, 1), (4, -1), (6, 1)), ((2, 1), (4, 1)), ((1, 1), (3, 1)), ((0, 1), (1, -1), (2, 1), (5, 1)))


def _lin(terms, get):
    acc = get(terms[0][0])
    for idx, sign in terms[1:]:
        a, b = acc.astype(f32), get(idx).astype(f32)
        acc = a + b if sign > 0 else a - b
    return acc


class _Memo(dict):
    def __init__(self, fn):
        super().__init__()
        self.fn = fn

    def __missing__(self, key):
        self[key] = val = self.fn(*key)
        return val


def _rc(o, i):
    return 2 * (o // 2) + i // 2, 2 * (o % 2) + i % 2


def _operand_fn(table, leaf):
    leaves = _Memo(leaf)
    mids = _Memo(lambda r1, i: _lin(table[r1], lambda o: leaves[_rc(o, i)]))
    return lambda r1, r2: _lin(table[r2], lambda i: mids[r1, i]).astype(bf16)


class _Combine:
    def __init__(self, style, emit):
        self.style, self.emit = style, emit
        self.vals, self.acc, self.used = {}, [None] * 4, [0] * 4

    def add(self, r, val):
        self.vals[r] = val
        for o, terms in enumerate(OUT):
            signs = dict(terms)
            if r not in signs:
                continue
            have = [t for t in signs if t in self.vals]
            n = len(terms)
            if len(have) == n or self.style == "eager" or (self.style == "hybrid" and len(have) == n - 1):
                todo = [t for t in have if not (self.used[o] >> t) & 1]
                todo.sort(key=lambda t: (t == r, -signs[t]))
                for t in todo:
                    if self.acc[o] is None:
                        if signs[t] < 0:
                            continue
                        self.acc[o] = self.vals[t]
                    else:
                        self.acc[o] = self.acc[o] + self.vals[t] if signs[t] > 0 else self.acc[o] - self.vals[t]
                    self.used[o] |= 1 << t
                if len(have) == n:
                    self.emit(o, self.acc[o])


def _strassen2(lhs, rhs, emit, style, order=range(7)):
    outer = [_Combine(style, lambda o, val, i=i: emit(*_rc(o, i), val)) for i in range(4)]
    for r1 in order:
        inner = _Combine(style, lambda i, val: outer[i].add(r1, val))
        for r2 in order:
            b = rhs(r1, r2)
            inner.add(r2, _dot(lhs(r1, r2), b))


def make(TQ=512, KC=128, LAG=4, GM=512, scopes=False, phases="pafd", fstyle="hybrid", pstyle="hybrid", dstyle="hybrid",
         forder=(1, 4, 0, 2, 3, 5, 6), porder=(1, 4, 0, 2, 3, 5, 6), dorder=(1, 4, 0, 2, 3, 5, 6), dorder2=(1, 4, 0, 2, 3, 5, 6), DK=256, DS=32):
    RB = TQ // 4

    def scope(name):
        return jax.named_scope(name) if scopes else contextlib.nullcontext()

    def kernel(x_hbm, wq_hbm, wkT_hbm, wvT_hbm, wo_hbm, wg_hbm, wu_hbm, wd_hbm, gw_hbm, o_hbm,
               wo_sc, wd_sc, oT_sc, sems, osems):
        S, D = x_hbm.shape
        Dh = D // H
        F = wd_sc.shape[0]
        NQ = S // TQ
        DQ = D // 4
        SQ = S // 4
        NG = F // 512
        V = pltpu.VMEM

        def attention(wg_sc, wu_sc, g_sc, xop_sc, x_sc, wq_sc, wkv_sc, gw_sc, k_sc, vT_sc, qT_sc, gT_sc, s_sc, m_sc):
            def xcp(c):
                return pltpu.make_async_copy(x_hbm.at[pl.ds(c * TQ, TQ)], x_sc.at[c % 2], sems.at[c % 2])
            first = [pltpu.make_async_copy(a, b, sems.at[2 + i]) for i, (a, b) in enumerate(
                [(wq_hbm, wq_sc), (wkT_hbm, wkv_sc.at[0]), (wvT_hbm, wkv_sc.at[1]), (gw_hbm, gw_sc)])]
            rest = [pltpu.make_async_copy(a, b, sems.at[6 + i]) for i, (a, b) in enumerate(
                [(wg_hbm, wg_sc), (wu_hbm, wu_sc), (wd_hbm, wd_sc), (wo_hbm, wo_sc)])]
            with scope("wait"):
                xcp(0).start()
                for c in first:
                    c.start()
                for c in first:
                    c.wait()

            def proj_body(c, carry):
                xcp(c).wait()

                @pl.when(c + 1 < NQ)
                def _():
                    xcp(c + 1).start()

                @pl.when(c + 1 == NQ)
                def _():
                    for cp in rest:
                        cp.start()
                x_ref = x_sc.at[c % 2]
                p0 = pl.multiple_of(c * RB, RB)
                wkv = jnp.concatenate([wkv_sc[0], wkv_sc[1]], axis=0)
                kvT = lax.dot_general(wkv, x_ref[...], NT, preferred_element_type=f32)
                k_sc[pl.ds(pl.multiple_of(c * TQ, TQ), TQ), :] = kvT[:Dh].T.astype(bf16)
                vT_sc[c] = kvT[Dh:].astype(bf16)
                xop = _operand_fn(LHS, lambda r, k: x_ref[r * RB:(r + 1) * RB, k * DQ:(k + 1) * DQ])

                def lhs(r1, r2):
                    op = xop(r1, r2)
                    xop_sc[7 * r1 + r2, pl.ds(pl.multiple_of(c * RB // 2, RB // 2), RB // 2), :] = pltpu.bitcast(op, u32)
                    return op

                def emit(r, j, val):
                    qT_sc[c, j * DQ:(j + 1) * DQ, r * RB:(r + 1) * RB] = (val * (Dh ** -0.5 * LOG2E)).astype(bf16).T
                if "p" in phases:
                    gw = gw_sc[...].astype(f32)
                    for r in range(4):
                        z = jnp.sum(x_ref[r * RB:(r + 1) * RB, :].astype(f32) * gw, axis=-1, keepdims=True)
                        g = jnp.broadcast_to(1.0 / (1.0 + jnp.exp(-z)), (RB, 128))
                        g_sc[r, pl.ds(p0, RB), :] = 1.0 - g
                        gT_sc[c, :, r * RB:(r + 1) * RB] = g.T[:8]
                    _strassen2(lhs, _operand_fn(RHS, lambda k, j: wq_sc[k * DQ:(k + 1) * DQ, j * DQ:(j + 1) * DQ]),
                               emit, pstyle, porder)
                return carry
            with scope("proj"):
                lax.fori_loop(0, NQ, proj_body, 0)

            def unit(cur, nxt, slot):
                if nxt is not None:
                    q = qT_sc[nxt[1], pl.ds(pl.multiple_of(nxt[0] * Dh, Dh), Dh), :]
                if cur is not None:
                    m = m_sc[slot]
                mx = l = o = None
                for c in range(S // KC):
                    sl = slice(c * KC, (c + 1) * KC)
                    if cur is not None:
                        p = jnp.exp2(s_sc[slot, sl, :].reshape(KC // 8, 8, TQ) - m[None])
                    if nxt is not None:
                        s = _dot(k_sc[sl, :], q)
                        mc = jnp.max(s.reshape(KC // 8, 8, TQ), axis=0)
                        mx = mc if mx is None else jnp.maximum(mx, mc)
                    if cur is not None:
                        lc = jnp.sum(p, axis=0)
                        l = lc if l is None else l + lc
                        oc = _dot(vT_sc[c * KC // TQ, :, c * KC % TQ:c * KC % TQ + KC], p.reshape(KC, TQ).astype(bf16))
                        o = oc if o is None else o + oc
                    if nxt is not None:
                        s_sc[slot, sl, :] = s
                if nxt is not None:
                    m_sc[slot] = jnp.broadcast_to(jnp.max(mx, axis=0, keepdims=True), (8, TQ))
                if cur is not None:
                    w = gT_sc[cur[1], 0:1, :] / jnp.sum(l, axis=0, keepdims=True)
                    oT_sc[cur[1], pl.ds(pl.multiple_of(cur[0] * Dh, Dh), Dh), :] = o * w

            def att_body(h, carry):
                for r in range(NQ):
                    u = r - LAG
                    unit((h, u) if u >= 0 else (h - 1, u + NQ), (h, r), r % LAG)
                return carry
            if "a" in phases:
                with scope("fill"):
                    for u in range(LAG):
                        unit(None, (0, u), u)
                    for u in range(NQ - LAG):
                        unit((0, u), (0, u + LAG), u % LAG)
                with scope("att"):
                    lax.fori_loop(1, H, att_body, 0)
                with scope("drain"):
                    for u in range(NQ - LAG, NQ):
                        unit((H - 1, u), None, u % LAG)
            for c in rest:
                c.wait()

        def gate_up(wg_sc, wu_sc, g_sc, xop_sc, hop_sc):
            NM = SQ // GM

            def ffn_body(it, carry):
                j = it // NM
                rows = pl.ds(pl.multiple_of((it % NM) * GM, GM), GM)
                prow = pl.ds(pl.multiple_of((it % NM) * (GM // 2), GM // 2), GM // 2)

                def wpair(k, n1):
                    cols = pl.ds(pl.multiple_of(j * 512 + n1 * 256, 256), 256)
                    return wg_sc[k * DQ:(k + 1) * DQ, cols].astype(f32), wu_sc[k * DQ:(k + 1) * DQ, cols].astype(f32)
                pairs = _Memo(wpair)

                def wleaf(k, n):
                    lanes = slice(n % 2 * 128, n % 2 * 128 + 128)
                    return jnp.concatenate([w[:, lanes] for w in pairs[k, n // 2]], axis=1)
                hblk, done = {}, set()
                hop = _operand_fn(LHS, lambda r, k: hblk[r, k])

                def emit(r, n, val):
                    hblk[r, 3 - n] = jnp.maximum(val[:, :128], 0.0) * val[:, 128:] * g_sc[r, rows, :]
                    for r1 in range(7):
                        for r2 in range(7):
                            if (r1, r2) not in done and all(_rc(o, i) in hblk for o, _ in LHS[r1] for i, _ in LHS[r2]):
                                done.add((r1, r2))
                                hop_sc[r1, r2, j, prow, :] = pltpu.bitcast(hop(r1, r2), u32)
                _strassen2(lambda r1, r2: pltpu.bitcast(xop_sc[7 * r1 + r2, prow, :], bf16),
                           _operand_fn(RHS, wleaf), emit, fstyle, forder)
                return carry
            if "f" in phases:
                with scope("ffn"):
                    lax.fori_loop(0, NG * NM, ffn_body, 0)

        def down(hop_sc, acc_sc, out_sc):
            def pick(table, r1):
                vals = []
                for col in zip(*table):
                    v = col[0]
                    for r in range(1, 7):
                        if col[r] != col[r - 1]:
                            v = jnp.where(r1 >= r, col[r], v)
                    vals.append(v)
                return vals

            def two(terms):
                return (terms[0][0], terms[-1][0], float(terms[1][1]) if len(terms) > 1 else 0.0)

            def ocps(o, i):
                r, n = 2 * (o // 2) + i // 2, 2 * (o % 2) + i % 2
                return [pltpu.make_async_copy(
                    out_sc[i].at[o, pl.ds(c * RB, RB)],
                    o_hbm.at[pl.ds(c * TQ + r * RB, RB), pl.ds(pl.multiple_of(n * DQ, DQ), DQ)], osems.at[0])
                    for c in range(NQ)]
            fin = []
            for n, r in enumerate(dorder):
                full = [o for o, terms in enumerate(OUT) if r in dict(terms) and all(t in dorder[:n + 1] for t, _ in terms)]
                assert len(full) == (n >= 3)
                rest_terms = [(dorder.index(t), float(sg)) for t, sg in OUT[full[0]] if t != r] if full else []
                assert not full or dict(OUT[full[0]])[r] == 1
                rest_terms += [(0, 0.0)] * (3 - len(rest_terms))
                fin.append((r, full[0] if full else 0) + sum(rest_terms, ()))
            for i in range(4):
                acc_sc[i][0] = jnp.zeros(acc_sc[i].shape[1:], f32)

            def down_body(n, carry):
                a0, a1, ac = pick([two(LHS[r]) for r in dorder], n)
                b0, b1, bc = pick([two(RHS[r]) for r in dorder], n)
                r1, c0, i0, k0, i1, k1, i2, k2 = pick(fin, n)

                def oT(o, i):
                    krow = pl.ds(pl.multiple_of((2 * (o % 2) + i % 2) * DQ, DQ), DQ)
                    lanes = pl.ds(pl.multiple_of((2 * (o // 2) + i // 2) * RB, RB), RB)
                    return jnp.concatenate([oT_sc[c, krow, lanes] for c in range(NQ)], axis=1)
                omid = _Memo(lambda i: (oT(a0, i) + ac * oT(a1, i)).T)

                def wblk(o, i, t):
                    k = 2 * (o // 2) + i // 2
                    cols = pl.ds(pl.multiple_of((2 * (o % 2) + i % 2) * DQ, DQ), DQ)
                    if t < NG:
                        return wd_sc[pl.ds(pl.multiple_of(t * 512 + (3 - k) * 128, 128), 128), cols].astype(f32)
                    return wo_sc[pl.ds(pl.multiple_of(k * DQ + (t - NG) * 128, 128), 128), cols].astype(f32)
                wmid = _Memo(lambda i, t: wblk(b0, i, t) + bc * wblk(b1, i, t))

                def emit(i, val):
                    for t in range(0, SQ, DS):
                        rows = slice(t, t + DS)
                        part = k0 * acc_sc[i][i0, rows] + k1 * acc_sc[i][i1, rows] + k2 * acc_sc[i][i2, rows]
                        acc_sc[i][n, rows] = val[rows]
                        out_sc[i][c0, rows] = (part + val[rows]).astype(o_hbm.dtype)

                    @pl.when(n >= 3)
                    def _():
                        for cp in ocps(c0, i):
                            cp.start()
                inner = _Combine(dstyle, emit)
                for r2 in dorder2:
                    prod = None
                    NT_ = NG + DQ // 128
                    for t0 in range(0, NT_, DK // 128):
                        ts = range(t0, min(t0 + DK // 128, NT_))
                        b = jnp.concatenate([_lin(RHS[r2], lambda i: wmid[i, t]).astype(bf16) for t in ts], axis=0)
                        a = jnp.concatenate([
                            pltpu.bitcast(hop_sc[r1, r2, t], bf16) if t < NG else
                            _lin(LHS[r2], lambda i: omid[i,][:, (t - NG) * 128:(t - NG + 1) * 128]).astype(bf16)
                            for t in ts], axis=1)
                        d = _dot(a, b)
                        prod = d if prod is None else prod + d
                    inner.add(r2, prod)
                return carry
            if "d" in phases:
                with scope("down"):
                    lax.fori_loop(0, 7, down_body, 0)
                for o in range(4):
                    for i in range(4):
                        for cp in ocps(o, i):
                            cp.wait()

        def outer(hop_sc):
            def front(wg_sc, wu_sc, g_sc, xop_sc):
                pl.run_scoped(lambda *refs: attention(wg_sc, wu_sc, g_sc, xop_sc, *refs),
                              V((2, TQ, D), bf16), V((D, D), bf16), V((2, Dh, D), bf16), V((1, D), bf16),
                              V((S, Dh), bf16), V((NQ, Dh, TQ), bf16), V((NQ, D, TQ), bf16), V((NQ, 8, TQ), f32),
                              V((LAG, S, TQ), f32), V((LAG, 8, TQ), f32))
                gate_up(wg_sc, wu_sc, g_sc, xop_sc, hop_sc)
            pl.run_scoped(front, V((D, F), bf16), V((D, F), bf16), V((4, SQ, 128), f32), V((49, SQ // 2, DQ), u32))
            pl.run_scoped(lambda *refs: down(hop_sc, *refs), [V((7, SQ, DQ), f32)] * 4, [V((4, SQ, DQ), o_hbm.dtype)] * 4)
        pl.run_scoped(outer, V((7, 7, NG, SQ // 2, 128), u32))

    @jax.jit
    def fn(A_x, A_wq, A_wk, A_wv, A_wo, B_x, B_W_gate, B_W_up, B_W_down, gate_w):
        B, S, D = A_x.shape
        F = B_W_gate.shape[1]
        NQ = S // TQ
        hbm = pl.BlockSpec(memory_space=pl.ANY)
        args = (A_x.reshape(S, D), A_wq, A_wk.T, A_wv.T, A_wo, B_W_gate, B_W_up, B_W_down, gate_w.reshape(1, D))
        V = pltpu.VMEM
        out = pl.pallas_call(
            kernel,
            in_specs=[hbm] * 9,
            out_specs=hbm,
            out_shape=jax.ShapeDtypeStruct((S, D), A_x.dtype),
            scratch_shapes=[V((D, D), bf16), V((F, D), bf16), V((NQ, D, TQ), f32),
                            pltpu.SemaphoreType.DMA((10,)), pltpu.SemaphoreType.DMA((1,))],
            compiler_params=pltpu.CompilerParams(vmem_limit_bytes=127 * 1024 * 1024),
            name="gm_kernel",
        )(*args)
        return out.reshape(B, S, D)
    return fn


pallas_gated_mix__grouped_kv_mqa__glu_gated_reglu__prompt_kernel = make(forder=(4,2,1,3,0,5,6))
```

```python
import contextlib
import jax
import jax.numpy as jnp
import numpy as np
from jax import lax
import jax.experimental.pallas as pl
import jax.experimental.pallas.tpu as pltpu

H = 32
LOG2E = float(np.log2(np.e))
NT = (((1,), (1,)), ((), ()))
f32 = jnp.float32
bf16 = jnp.bfloat16
u32 = jnp.uint32


def _dot(a, b):
    return jnp.dot(a, b, preferred_element_type=f32)


LHS = (((0, 1), (3, -1)), ((2, 1), (3, -1)), ((0, 1),), ((3, 1),), ((1, 1), (0, -1)), ((2, 1), (0, -1)), ((1, 1), (3, -1)))
RHS = (((0, 1), (3, -1)), ((0, 1),), ((1, 1), (3, 1)), ((0, 1), (2, 1)), ((3, 1),), ((0, 1), (1, 1)), ((2, 1), (3, 1)))
OUT = (((0, 1), (3, 1), (4, -1), (6, 1)), ((2, 1), (4, 1)), ((1, 1), (3, 1)), ((0, 1), (1, -1), (2, 1), (5, 1)))


def _lin(terms, get):
    acc = get(terms[0][0])
    for idx, sign in terms[1:]:
        a, b = acc.astype(f32), get(idx).astype(f32)
        acc = a + b if sign > 0 else a - b
    return acc


def _tree(op, vals):
    vals = list(vals)
    while len(vals) > 1:
        vals = [op(*vals[i:i + 2]) if i + 1 < len(vals) else vals[i] for i in range(0, len(vals), 2)]
    return vals[0]


class _Memo(dict):
    def __init__(self, fn):
        super().__init__()
        self.fn = fn

    def __missing__(self, key):
        self[key] = val = self.fn(*key)
        return val


def _rc(o, i):
    return 2 * (o // 2) + i // 2, 2 * (o % 2) + i % 2


def _operand_fn(table, leaf):
    leaves = _Memo(leaf)
    mids = _Memo(lambda r1, i: _lin(table[r1], lambda o: leaves[_rc(o, i)]))
    return lambda r1, r2: _lin(table[r2], lambda i: mids[r1, i]).astype(bf16)


class _Combine:
    def __init__(self, emit):
        self.emit, self.vals = emit, {}

    def add(self, r, val):
        self.vals[r] = val
        for o, terms in enumerate(OUT):
            if r in dict(terms) and all(t in self.vals for t, _ in terms):
                seen = list(self.vals)
                terms = sorted(terms, key=lambda t: seen.index(t[0]))
                if terms[0][1] < 0:
                    terms[:2] = terms[1::-1]
                self.emit(o, _lin(terms, lambda t: self.vals[t]))


def _strassen2(lhs, rhs, emit, order, order2):
    outer = [_Combine(lambda o, val, i=i: emit(*_rc(o, i), val)) for i in range(4)]
    for n, r1 in enumerate(order):
        inner = _Combine(lambda i, val: outer[i].add(r1, val))
        for r2 in (order2[n] if isinstance(order2[0], tuple) else order2):
            b = rhs(r1, r2)
            inner.add(r2, _dot(lhs(r1, r2), b))


def make(TQ=512, KC=128, scopes=False, phases="fad",
         forder=(4, 2, 1, 3, 0, 5, 6), forder2='4123056 4123056 4213065 4120356 4123056 4123056 0423165', porder=(2, 4, 3, 6, 0, 1, 5), porder2='4213056 2046135 4102635 4132506 2610345 2514306 1432065',
         dorder=(1, 4, 0, 2, 3, 5, 6), DKS=(5, 4), DS=64, sched='Q2 Q1 P1 Q0 P2 P0 R12 Q3 S10 S12 R01 S01 S21 R02 P3 S20 R13 R23 S32 S02 R03 S23 S13 S31 S03 S30', T4=(-1.375, 0.375, -0.375, 1.375), ROT=(0, 1, 3, 1, 3, 2, 2),
         KVAT=((5, 0), (5, 4), (6, 0), (6, 4)), SROWS=0, VL=128, FINE=True, PRIO=0, LAST=(5, 0), NF=5, FW='1998658 8703644 6888668 7702534 6846566 8835410 6756633', NV=4, LO=16, cp=None):

    forder2 = [tuple(map(int, w)) for w in forder2.split()]
    porder2 = [tuple(map(int, w)) for w in porder2.split()]
    if isinstance(FW, str): FW = [int(c) for c in FW.replace(" ", "")]

    def scope(name):
        return jax.named_scope(name) if scopes else contextlib.nullcontext()

    def kernel(x_hbm, wq_hbm, wkT_hbm, wvT_hbm, wo_hbm, wg_hbm, wu_hbm, wd_hbm, gw_hbm, o_hbm,
               k_sc, vT_sc, qT_sc, gT_sc, hop_sc, sems, wsems, osems):
        S, D = x_hbm.shape
        Dh = D // H
        F = wd_hbm.shape[0]
        NQ = S // TQ
        DQ = D // 4
        SQ = S // 4
        NG = F // 512
        V = pltpu.VMEM

        def wcopies(wg_sc, wu_sc, j):
            cols = pl.ds(pl.multiple_of(j * 512, 512), 512)
            return [pltpu.make_async_copy(src.at[:, cols], dst.at[j % 2], wsems.at[i, j % 2])
                    for i, (src, dst) in enumerate([(wg_hbm, wg_sc), (wu_hbm, wu_sc)])]

        def project(g_sc, xop_sc, x_sc, wq_sc, wkv_sc, gw_sc):
            def part(x, r0, r1, c0, c1):
                idx = (pl.ds(r0, r1 - r0), pl.ds(c0, c1 - c0))
                return ((x_hbm, x_sc) if x else (wq_hbm, wq_sc)), idx
            stages = {
                (0, 0): [part(0, 0, D, 768, D), part(1, 0, 512, 0, 512)],
                (0, 2): [part(0, 0, D, 512, 768), part(1, 512, 1024, 0, 512)],
                (1, 0): [part(1, 0, 1024, 512, D)],
                (2, 0): [part(0, 0, D, 0, 512), part(1, 1024, S, 512, D)],
                LAST: [part(1, 1024, S, 0, 512),
                         ((wkT_hbm, wkv_sc.at[0]), ...), ((wvT_hbm, wkv_sc.at[1]), ...), ((gw_hbm, gw_sc.at[0:D // 128]), ...)],
            }
            if not FINE:
                stages[0, 0] += stages.pop((0, 2))
            slot = iter(range(11))
            need = {at: [pltpu.make_async_copy(src.at[idx], dst.at[idx], sems.at[next(slot)]) for (src, dst), idx in parts]
                    for at, parts in stages.items()}
            for cps in need.values():
                for cp in cps:
                    cp.start(priority=PRIO)
            xop = _operand_fn(LHS, lambda r, k: x_sc[r * SQ:(r + 1) * SQ, k * DQ:(k + 1) * DQ])
            wop = _operand_fn(RHS, lambda k, j: wq_sc[k * DQ:(k + 1) * DQ, j * DQ:(j + 1) * DQ])

            def kv(c):
                gw = gw_sc[0:D // 128].astype(f32)
                gw = jnp.concatenate([jnp.broadcast_to(gw[t:t + 1], (16, 128)) for t in range(D // 128)], axis=1)
                wkv = jnp.concatenate([wkv_sc[0], wkv_sc[1], gw.astype(bf16)], axis=0)
                res = lax.dot_general(wkv, x_sc[c * TQ:(c + 1) * TQ, :], NT, preferred_element_type=f32)
                k_sc[c * TQ // 2:(c + 1) * TQ // 2, :] = pltpu.bitcast(res[:Dh].T.astype(bf16), u32)
                vT_sc[c] = pltpu.bitcast(res[Dh:2 * Dh].astype(bf16), u32)
                g = 1.0 / (1.0 + jnp.exp(-res[2 * Dh:2 * Dh + 8]))
                gT_sc[c] = g
                g_sc[c] = jnp.concatenate([1.0 - g] * 16, axis=0).T

            def rhs(r1, r2):
                at = (porder.index(r1), porder2[porder.index(r1)].index(r2))
                if at in need:
                    with scope("w%d%d" % at):
                        for cp in need.pop(at):
                            cp.wait()
                if (porder.index(r1), porder2[porder.index(r1)].index(r2)) in KVAT:
                    kv(KVAT.index((porder.index(r1), porder2[porder.index(r1)].index(r2))))
                return wop(r1, r2)

            def lhs(r1, r2):
                op = xop(r1, r2)
                xop_sc[7 * r1 + r2] = pltpu.bitcast(op, u32)
                return op

            def emit(r, j, val):
                qT_sc[r, j * DQ:(j + 1) * DQ, :] = (val * (Dh ** -0.5 * LOG2E)).astype(bf16).T
            with scope("proj"):
                _strassen2(lhs, rhs, emit, porder, porder2)

        def gate_up(wg_sc, wu_sc, g_sc, xop_sc, kb_sc, sf_sc, qu_sc):
            def ffn_body(j, carry):
                with scope("fw"):
                    for cp in wcopies(wg_sc, wu_sc, j):
                        cp.wait()

                @pl.when(j + 1 < NG)
                def _():
                    for cp in wcopies(wg_sc, wu_sc, j + 1):
                        cp.start()

                def wpair(k, n1):
                    return [w[j % 2, k * DQ:(k + 1) * DQ, n1 * 256:(n1 + 1) * 256].astype(f32) for w in (wg_sc, wu_sc)]
                pairs = _Memo(wpair)

                def wleaf(k, n):
                    lanes = slice(n % 2 * 128, n % 2 * 128 + 128)
                    return jnp.concatenate([w[:, lanes] for w in pairs[k, n // 2]], axis=1)
                hblk, done = {}, set()
                mids = _Memo(lambda r1, i: _lin(LHS[r1], lambda o: hblk[_rc(o, i)]))

                def emit(r, n, val):
                    hblk[r, 3 - n] = jnp.maximum(val[:, :128], 0.0) * val[:, 128:] * g_sc[r]
                    for r1 in range(7):
                        for i2, part in ((0, 0), (1, 0), (0, 1), (1, 1)):
                            if (r1, i2, part) not in done and all(
                                    _rc(o, 2 * i2 + k2) in hblk for o, _ in LHS[r1] for k2 in range(part + 1)):
                                done.add((r1, i2, part))
                                for half in range(2):
                                    i, rows = (2 * i2 + half + ROT[r1]) % 4, slice(half * SQ // 2, (half + 1) * SQ // 2)
                                    op = mids[r1, 2 * i2][rows]
                                    hop_sc[r1, part, i, j] = T4[i] * op + mids[r1, 2 * i2 + 1][rows] if part else op
                todo = [(u, g, t) for u in range(NU) for g in range(2 * NF) for t in LT]
                weight = [FW[a * 7 + b] for a in range(7) for b in range(7) for _ in range(SQ // 16)]
                marks = np.cumsum(weight) * len(todo) // sum(weight)

                def lhs(r1, r2):
                    first = (forder.index(r1) * 7 + forder2[forder.index(r1)].index(r2)) * (SQ // 16)
                    rows = []
                    for a in range(SQ // 16):
                        row = xop_sc[7 * r1 + r2, 8 * a:8 * a + 8]
                        for u, g, t in todo[marks[first + a - 1] if first + a else 0:marks[first + a]]:
                            val = vpu_scores(kb_sc.at[g], qu_sc.at[u], t)
                            unit = jnp.minimum(NQ + j * NU + u, H * NQ - 1)
                            sf_sc[unit % NQ, unit // NQ, 8 * g:8 * g + 8, t * 128:(t + 1) * 128] = val
                            row = jnp.concatenate([jnp.where(j < 0, pltpu.bitcast(val, u32), row[:, :128]), row[:, 128:]], axis=1)
                        rows.append(row)
                    return pltpu.bitcast(jnp.concatenate(rows, axis=0), bf16)
                _strassen2(lhs, _operand_fn(RHS, wleaf), emit, forder, forder2)
                if NF:
                    stage_units(qu_sc, j + 1)
                return carry
            if "f" in phases:
                with scope("ffn"):
                    lax.fori_loop(0, NG, ffn_body, 0)

        NC = S // KC
        VC = range(NC - NV, NC)
        FC = range(NC - NV - NF, NC - NV)
        ROW = [c * KC - 16 * sum(f < c for f in FC) for c in range(NC + 1)]
        SR = SROWS or -(-ROW[-1] // 32) * 32
        LT = range(TQ // 128)
        NU = -(-(H - 1) * NQ // NG)

        def q_rows(qb, h):
            return qT_sc[qb, pl.ds(pl.multiple_of(h * Dh, Dh), Dh), :]

        def vpu_scores(kb, q_ref, t):
            val = None
            for d in range(Dh):
                term = kb[d] * q_ref[d:d + 1, 128 * t:128 * t + 128]
                val = term if val is None else val + term
            return val

        def stage_units(qu_sc, j):
            for u in range(NU):
                unit = jnp.minimum(NQ + j * NU + u, H * NQ - 1)
                qu_sc[u] = q_rows(unit % NQ, unit // NQ).astype(f32)

        def attention(oT_sc, w_sc, wo_sc, wd_sc, s_sc, m_sc, kb_sc, qf_sc, sf_sc, fill):
            def sweep(h_cur, h_nxt, blocks):
                both = h_cur is not None and h_nxt is not None
                regs = [KC // 16 - (both and (c in VC or c in FC)) for c in range(NC)]
                slots = [(c, u) for c in range(NC) for u in range(regs[c])][LO:]
                todo = [(g, t) for g in range(2 * NV) for t in LT] if both else []
                tie = {slots[(a + 1) * len(slots) // len(todo) - 1]: piece for a, piece in enumerate(todo)}
                for qb in blocks:
                    extra = []
                    for c in range(NC):
                        start, stop = ROW[c], ROW[c + 1]
                        if h_cur is not None:
                            p = jnp.concatenate([s_sc[qb][t, start:stop] for t in LT], axis=1)
                            if c in FC:
                                p = jnp.concatenate([p, sf_sc[qb, h_cur, 16 * FC.index(c):16 * FC.index(c) + 16]], axis=0)
                            p = jnp.exp2(p.reshape(KC // 8, 8, TQ) - m_sc[qb][None])
                            part = _tree(jnp.add, [p[j] for j in range(KC // 8)])
                            den = part if c == 0 else den + part
                        if h_nxt is not None:
                            rows = []
                            for u in range(regs[c]):
                                row = k_sc[c * KC // 2 + 8 * u:c * KC // 2 + 8 * u + 8, :]
                                if (c, u) in tie:
                                    g, t = tie[c, u]
                                    val = vpu_scores(kb_sc.at[g], qf_sc.at[qb], t)
                                    extra.append((g, t, val))
                                    row = jnp.where(h_nxt < 0, pltpu.bitcast(val, u32)[:, :Dh], row)
                                rows.append(row)
                            s = _dot(pltpu.bitcast(jnp.concatenate(rows, axis=0), bf16), q_rows(qb, h_nxt))
                            for t in LT:
                                n = min(16 * regs[c], stop - start)
                                s_sc[qb][t, start:start + n] = s[:n, t * 128:(t + 1) * 128]
                            if c in FC and both:
                                s = jnp.concatenate([s, sf_sc[qb, h_nxt, 16 * FC.index(c):16 * FC.index(c) + 16]], axis=0)
                            elif c in FC:
                                sf_sc[qb, 0, 16 * FC.index(c):16 * FC.index(c) + 16] = s[KC - 16:]
                            part = jnp.max(s.reshape(-1, 8, TQ), axis=0)
                            top = part if c == 0 else jnp.maximum(top, part)
                        if h_cur is not None:
                            vT = vT_sc[c * KC // TQ, :, c * KC % TQ:c * KC % TQ + KC]
                            part = _dot(pltpu.bitcast(vT, bf16), p.reshape(KC, TQ).astype(bf16))
                            num = part if c == 0 else num + part
                    if h_cur is not None:
                        w_sc[qb, h_cur // (128 // Dh), pl.ds(h_cur % (128 // Dh), 1), :] = jnp.sum(den, axis=0, keepdims=True)
                        oT_sc[pl.ds(pl.multiple_of(qb * D + h_cur * Dh, Dh), Dh), :] = num
                    if h_nxt is not None:
                        tops = [[top[:, 128 * t:128 * t + 128]] for t in LT]
                        for g, t, val in extra:
                            row0 = ROW[VC[g // 2] + 1] - 16 + 8 * (g % 2)
                            s_sc[qb][t, row0:row0 + 8] = val
                            tops[t].append(val)
                        top = jnp.concatenate([_tree(jnp.maximum, v) for v in tops], axis=1)
                        m_sc[qb] = jnp.broadcast_to(jnp.max(top, axis=0, keepdims=True), (8, TQ))
                        if NV:
                            qf_sc[qb] = q_rows(qb, jnp.minimum(h_nxt + 1, H - 1)).astype(f32)

            def fill_body(r, carry):
                sweep(None, 0, [r])
                return carry

            HG = 128 // Dh

            def finish(r, grp):
                w = gT_sc[r, 0:1, :] / w_sc[r, grp, :HG]
                tile = oT_sc.at[pl.ds(pl.multiple_of(r * D + grp * 128, 128), 128)]
                o = jnp.concatenate([tile[t * Dh:(t + 1) * Dh, :] * w[t:t + 1] for t in range(HG)], axis=0)
                for b in range(0, TQ, 128):
                    tile[:, b:b + 128] = o[:, b:b + 128].T

            def att_body(h, carry):
                u = h - HG - 1
                finish(jnp.where(u < 0, NQ - 1, u % NQ), jnp.where(u < 0, H // HG, u // NQ))
                sweep(h - 1, h, range(NQ))
                return carry

            def drain_body(r, carry):
                sweep(H - 1, None, [r])
                finish(r, H // HG - 1)
            if fill:
                with scope("fill"):
                    sweep(None, 0, range(NQ))
                return
            w_sc[NQ - 1, H // HG] = jnp.ones(w_sc.shape[2:], f32)
            oT_sc[NQ * D:] = jnp.zeros((128, TQ), f32)
            late = [pltpu.make_async_copy(a, b, sems.at[11 + i]) for i, (a, b) in enumerate([(wd_hbm, wd_sc), (wo_hbm, wo_sc)])]
            for cp in late:
                cp.start()
            if "a" in phases:
                with scope("att"):
                    lax.fori_loop(1, H, att_body, 0)
            for cp in late:
                cp.wait()
            if "a" in phases:
                with scope("drain"):
                    finish(NQ - 1, H // HG - 2)
                    for r in range(NQ):
                        drain_body(r, 0)

        def down(oT_sc, w_sc, wo_sc, wd_sc, acc_sc, out_sc):
            def pick(table, step):
                vals = []
                for col in zip(*table):
                    v = col[0]
                    for r in range(1, 7):
                        if col[r] != col[r - 1]:
                            v = jnp.where(step >= r, col[r], v)
                    vals.append(v)
                return vals

            def two(terms):
                return divmod(terms[0][0], 2) + divmod(terms[-1][0], 2) + (float(terms[1][1]) if len(terms) > 1 else 0.0,)

            RB = S // 8

            def staged(o, i):
                return out_sc.at[o, pl.ds(pl.multiple_of(i * RB, RB), RB)]

            def ocp(o, i):
                rows = pl.ds(pl.multiple_of((4 * (o // 2) + i) * RB, RB), RB)
                cols = pl.ds(pl.multiple_of((o % 2) * 512, 512), 512)
                return pltpu.make_async_copy(staged(o, i), o_hbm.at[rows, cols], osems.at[0])
            fin = []
            for n, r in enumerate(dorder):
                full = [o for o, terms in enumerate(OUT) if r in dict(terms) and all(t in dorder[:n + 1] for t, _ in terms)]
                assert len(full) == (n >= 3)
                others = [(dorder.index(t), float(sg)) for t, sg in OUT[full[0]] if t != r] if full else []
                assert not full or dict(OUT[full[0]])[r] == 1
                others += [(0, 0.0)] * (3 - len(others))
                fin.append((r, ROT[r], full[0] if full else 0) + sum(others, ()))


            def down_body(n, carry):
                *ablk, ac = pick([two(LHS[r]) for r in dorder], n)
                *bblk, bc = pick([two(RHS[r]) for r in dorder], n)
                r1, rot, c0, i0, k0, i1, k1, i2, k2 = pick(fin, n)
                phys = [(i + 4 - rot) & 3 for i in range(4)]

                def oblk(row, col, i, half, u):
                    ref = oT_sc.at[pl.ds(pl.multiple_of((2 * row + (phys[i] >> 1)) * D + (2 * col + half) * DQ, DQ), DQ),
                                   pl.ds(pl.multiple_of((phys[i] & 1) * RB, RB), RB)]
                    return jnp.concatenate([ref[u * 128:(u + 1) * 128, b:b + 128] for b in range(0, RB, 128)], axis=0)
                omid = _Memo(lambda *idx: oblk(*ablk[:2], *idx) + ac * oblk(*ablk[2:], *idx))
                hop = hop_sc.at[r1]
                alpha = _Memo(lambda i, t: hop[0, i, t] if t < NG else omid[i, 0, t - NG])
                beta = _Memo(lambda i, t: hop[1, i, t] if t < NG else T4[i] * omid[i, 0, t - NG] + omid[i, 1, t - NG])

                def wblk(row, col, half, j, t):
                    cols = pl.ds(pl.multiple_of(col * 512, 512), 512)
                    if t < NG:
                        ref, top = wd_sc.at[pl.ds(pl.multiple_of((1 - row) * 256, 256), F - 256), cols], t * 512 + (1 - half) * 128
                    else:
                        ref, top = wo_sc.at[pl.ds(pl.multiple_of(row * 512, 512), 512), cols], half * DQ + (t - NG) * 128
                    return ref[top:top + 128, j * 128:(j + 1) * 128].astype(f32)
                wmid = _Memo(lambda *idx: wblk(*bblk[:2], *idx) + bc * wblk(*bblk[2:], *idx))
                gamma = _Memo(lambda j, t: wmid[0, j, t] - T4[j] * wmid[1, j, t])

                def emit(i, j, val):
                    for t in range(0, RB, DS):
                        rows = slice(t, t + DS)
                        acc = lambda slot: acc_sc[j].at[phys[i], pl.ds(pl.multiple_of(slot * RB, RB), RB)]
                        part = k0 * acc(i0)[rows] + k1 * acc(i1)[rows] + k2 * acc(i2)[rows]
                        acc(n)[rows] = val[rows]
                        staged(c0, phys[i])[rows, j * 128:(j + 1) * 128] = (jnp.where(n > 0, part, 0.0) + val[rows]).astype(o_hbm.dtype)

                    if all((i, z) in done for z in range(4)):
                        @pl.when(n >= 3)
                        def _():
                            ocp(c0, phys[i]).start()

                def product(lhs, rhs):
                    res, t0 = [], 0
                    for width in DKS:
                        ts = range(t0, t0 + width)
                        t0 += width
                        b = jnp.concatenate([rhs(t) for t in ts], axis=0).astype(bf16)
                        res.append(_dot(jnp.concatenate([lhs(t) for t in ts], axis=1).astype(bf16), b))
                    return _tree(jnp.add, res)

                def scaled(c, v):
                    return v if c == 1 else c * v
                rho = _Memo(lambda lo, hi, t: scaled(1 / (T4[hi] - T4[lo]), beta[lo, t] - beta[hi, t]))
                sig = _Memo(lambda lo, hi, t: gamma[lo, t] + gamma[hi, t])
                got, done = {}, set()
                for name in sched.split():
                    i, j = int(name[1]), int(name[-1])
                    lo, hi = min(i, j), max(i, j)
                    if name[0] == "P":
                        got[name] = product(lambda t: alpha[i, t], lambda t: gamma[i, t])
                    elif name[0] == "Q":
                        got[name] = product(lambda t: beta[i, t], lambda t: wmid[1, i, t])
                    elif name[0] == "R":
                        got[name] = product(lambda t: rho[lo, hi, t], lambda t: sig[lo, hi, t])
                    else:
                        step = jnp.add if i < j else jnp.subtract
                        got[name] = product(lambda t: alpha[i, t] + rho[lo, hi, t],
                                            lambda t: step(sig[lo, hi, t], scaled(T4[hi] - T4[lo], wmid[1, j, t])))
                    for i in range(4):
                        for j in range(4):
                            need = [f"P{i}", f"Q{j}"] + ([f"R{min(i, j)}{max(i, j)}", f"S{i}{j}"] if i != j else [])
                            if (i, j) not in done and all(x in got for x in need):
                                done.add((i, j))
                                v = [got[x] for x in need]
                                emit(i, j, v[0] + v[1] if i == j else v[3] + (v[1] - v[0] - v[2]))
                return carry
            if "d" in phases:
                with scope("down"):
                    lax.fori_loop(0, 7, down_body, 0)
            pltpu.make_async_copy(o_hbm, o_hbm, osems.at[0]).wait()

        def middle(s_sc, *att):
            def feed_forward(keep, wg_sc, wu_sc, kf_sc, qu_sc):
                for cp in wcopies(wg_sc, wu_sc, 0):
                    cp.start()
                for ref, chunks in ((kf_sc, FC), (att[1], VC)):
                    for i, c in enumerate(chunks):
                        kf = pltpu.bitcast(k_sc[(c + 1) * KC // 2 - 8:(c + 1) * KC // 2, :], bf16).astype(f32)
                        for d in range(Dh):
                            col = jnp.broadcast_to(kf[:, d:d + 1], (16, 128))
                            ref[2 * i, d] = col[:8]
                            ref[2 * i + 1, d] = col[8:]
                stage_units(qu_sc, 0)
                attention(None, None, None, None, s_sc, *att, True)
                gate_up(wg_sc, wu_sc, *keep, kf_sc, att[3], qu_sc)

            def front(*keep):
                pl.run_scoped(lambda *refs: project(*keep, *refs),
                              V((S, D), bf16), V((D, D), bf16), V((2, Dh, D), bf16), V((64, 128), bf16))
                pl.run_scoped(lambda *refs: feed_forward(keep, *refs), V((2, D, 512), bf16), V((2, D, 512), bf16),
                              V((2 * NF, Dh, 8, 128), f32), V((NU, Dh, TQ), f32))
            pl.run_scoped(front, V((4, SQ, 128), f32), V((49, SQ // 2, DQ), u32))

            def back(*keep):
                attention(*keep, s_sc, *att, False)
                down(*keep, s_sc, qT_sc)
            pl.run_scoped(back, V((NQ * D + 128, TQ), f32), V((NQ, D // 128 + 1, 8, TQ), f32), V((D, D), bf16), V((F, D), bf16))
        pl.run_scoped(middle, [V((TQ // 128, SR, 128), f32)] * NQ, V((NQ, 8, TQ), f32), V((2 * NV, Dh, 8, 128), f32),
                      V((NQ, Dh, TQ), f32), V((NQ, H, 16 * NF, TQ), f32))

    @jax.jit
    def fn(A_x, A_wq, A_wk, A_wv, A_wo, B_x, B_W_gate, B_W_up, B_W_down, gate_w):
        B, S, D = A_x.shape
        Dh = D // H
        F = B_W_gate.shape[1]
        NQ = S // TQ
        hbm = pl.BlockSpec(memory_space=pl.ANY)
        args = (A_x.reshape(S, D), A_wq, A_wk.T, A_wv.T, A_wo, B_W_gate, B_W_up, B_W_down, gate_w.reshape(D // 128, 128))
        V = pltpu.VMEM
        out = pl.pallas_call(
            kernel,
            in_specs=[hbm] * 9,
            out_specs=hbm,
            out_shape=jax.ShapeDtypeStruct((S, D), A_x.dtype),
            scratch_shapes=[V((S // 2, Dh), u32), V((NQ, Dh // 2, TQ), u32),
                            V((NQ, D, TQ), bf16), V((NQ, 8, TQ), f32), V((7, 2, 4, F // 512, S // 8, 128), f32),
                            pltpu.SemaphoreType.DMA((13,)), pltpu.SemaphoreType.DMA((2, 2)), pltpu.SemaphoreType.DMA((1,))],
            compiler_params=pltpu.CompilerParams(vmem_limit_bytes=VL * 1024 * 1024, **(cp or {})),
            name="gm_kernel",
        )(*args)
        return out.reshape(B, S, D)
    return fn


pallas_gated_mix__grouped_kv_mqa__glu_gated_reglu__prompt_kernel = make()
```

```python
import jax
import jax.numpy as jnp
import numpy as np
from jax import lax
import jax.experimental.pallas as pl
import jax.experimental.pallas.tpu as pltpu

f32, bf16, u32 = jnp.float32, jnp.bfloat16, jnp.uint32

S, D, F, H = 2048, 1024, 3584, 32
DH = D // H
TQ = 512
NQ = S // TQ
KC = 128
NC = S // KC
LANES = range(TQ // 128)
HG = 128 // DH
HU = 2
NG = F // 512
DQ = D // 4
RB = S // 8
Q_SCALE = DH ** -0.5 * float(np.log2(np.e))

NF, NV = 5, 8
FC, VC = range(NF), range(NC - NV, NC)
NU = -(-(H - HU) * NQ // NG)

LHS = (((0, 1), (3, -1)), ((2, 1), (3, -1)), ((0, 1),), ((3, 1),),
       ((1, 1), (0, -1)), ((2, 1), (0, -1)), ((1, 1), (3, -1)))
RHS = (((0, 1), (3, -1)), ((0, 1),), ((1, 1), (3, 1)), ((0, 1), (2, 1)),
       ((3, 1),), ((0, 1), (1, 1)), ((2, 1), (3, 1)))
OUT = (((0, 1), (3, 1), (4, -1), (6, 1)), ((2, 1), (4, 1)), ((1, 1), (3, 1)),
       ((0, 1), (1, -1), (2, 1), (5, 1)))

T4 = (-1.375, 0.375, -0.375, 1.375)
ROT = (0, 1, 3, 1, 3, 2, 2)


def _order(outer, inner):
    return tuple((int(r1), tuple(map(int, word))) for r1, word in zip(outer, inner.split()))


PROJ_ORDER = _order("2436015", "4213056 2046135 4102635 4132506 2610345 2514306 1432065")
FFN_ORDER = _order("4213056", "4123056 4123056 4213065 4120356 4123056 4123056 0423165")
FFN_SHARE = [int(c) for c in "1898658 8503644 6988668 7710544 6946566 8835520 5756633" if c != " "]
DOWN_OUTER = (1, 4, 0, 2, 3, 5, 6)
DOWN_INNER = "Q2 Q1 P1 Q0 P2 P0 S10 Q3 R12 S21 R01 S01 S12 R02 P3 S20 R13 S32 R03 S03 R23 S23 S30 S13 S31 S02"


def _dot(a, b):
    return jnp.dot(a, b, preferred_element_type=f32)


def _ds(start, size, align):
    return pl.ds(start if isinstance(start, int) else pl.multiple_of(start, align), size)


def _lin(terms, get):
    acc = get(terms[0][0])
    for idx, sign in terms[1:]:
        a, b = acc.astype(f32), get(idx).astype(f32)
        acc = a + b if sign > 0 else a - b
    return acc


def _tree_sum(vals):
    while len(vals) > 1:
        vals = [vals[i] + vals[i + 1] if i + 1 < len(vals) else vals[i] for i in range(0, len(vals), 2)]
    return vals[0]


class _Memo(dict):
    def __init__(self, fn):
        super().__init__()
        self.fn = fn

    def __missing__(self, key):
        self[key] = val = self.fn(*key)
        return val


def _rc(outer, inner):
    return 2 * (outer // 2) + inner // 2, 2 * (outer % 2) + inner % 2


def _operands(table, leaf):
    leaves = _Memo(leaf)
    mids = _Memo(lambda r1, i: _lin(table[r1], lambda o: leaves[_rc(o, i)]))
    return lambda r1, r2: _lin(table[r2], lambda i: mids[r1, i]).astype(bf16)


class _Combine:
    def __init__(self, emit):
        self.emit, self.vals = emit, {}

    def add(self, r, val):
        self.vals[r] = val
        for o, terms in enumerate(OUT):
            if r in dict(terms) and all(t in self.vals for t, _ in terms):
                arrival = list(self.vals)
                terms = sorted(terms, key=lambda t: arrival.index(t[0]))
                if terms[0][1] < 0:
                    terms[:2] = terms[1::-1]
                self.emit(o, _lin(terms, lambda t: self.vals[t]))


def _strassen2(order, operands, emit):
    outer = [_Combine(lambda o, val, i=i: emit(*_rc(o, i), val)) for i in range(4)]
    for n, (r1, inner_order) in enumerate(order):
        inner = _Combine(lambda i, val: outer[i].add(r1, val))
        for m, r2 in enumerate(inner_order):
            inner.add(r2, _dot(*operands((n, m), r1, r2)))


def _vpu_scores(k_ref, q_ref, g, t):
    val = None
    for d in range(DH):
        term = k_ref[g, d] * q_ref[d:d + 1, 128 * t:128 * (t + 1)]
        val = term if val is None else val + term
    return val


def _tie(never, val, operand):
    return jnp.where(never, pltpu.bitcast(val, u32)[:, :operand.shape[1]], operand)


def _kernel(x_hbm, wq_hbm, wkT_hbm, wvT_hbm, wo_hbm, wg_hbm, wu_hbm, wd_hbm, gw_hbm, o_hbm,
            k_sc, vT_sc, qT_sc, gT_sc, h_sc, p_sc, kv_sc, sf_sc, sems, wsems, osem):
    V = pltpu.VMEM

    def q_rows(qb, h):
        return qT_sc[qb, _ds(h * DH, DH, DH), :]

    def project(g_sc, xop_sc, x_sc, wq_sc, wkv_sc, gw_sc):
        def x_part(r0, r1, c0, c1):
            return x_hbm.at[r0:r1, c0:c1], x_sc.at[r0:r1, c0:c1]

        def w_part(c0, c1):
            return wq_hbm.at[:, c0:c1], wq_sc.at[:, c0:c1]

        stages = {
            (0, 0): [w_part(768, D), x_part(0, 512, 0, 512)],
            (0, 2): [w_part(512, 768), x_part(512, 1024, 0, 512)],
            (1, 0): [x_part(0, 1024, 512, D)],
            (2, 0): [w_part(0, 512), x_part(1024, S, 512, D)],
            (5, 0): [x_part(1024, S, 0, 512), (wkT_hbm, wkv_sc.at[0]), (wvT_hbm, wkv_sc.at[1]),
                     (gw_hbm, gw_sc.at[0:D // 128])],
        }
        slot = iter(range(11))
        copies = {at: [pltpu.make_async_copy(src, dst, sems.at[next(slot)]) for src, dst in parts]
                  for at, parts in stages.items()}
        for group in copies.values():
            for copy in group:
                copy.start()

        def kv_gate(c):
            gw = gw_sc[0:D // 128].astype(f32)
            gw = jnp.concatenate([jnp.broadcast_to(gw[t:t + 1], (16, 128)) for t in range(D // 128)], axis=1)
            w = jnp.concatenate([wkv_sc[0], wkv_sc[1], gw.astype(bf16)], axis=0)
            res = lax.dot_general(w, x_sc[c * TQ:(c + 1) * TQ, :], (((1,), (1,)), ((), ())),
                                  preferred_element_type=f32)
            k_sc[c * TQ // 2:(c + 1) * TQ // 2, :] = pltpu.bitcast(res[:DH].T.astype(bf16), u32)
            vT_sc[c] = pltpu.bitcast(res[DH:2 * DH].astype(bf16), u32)
            g = 1.0 / (1.0 + jnp.exp(-res[2 * DH:2 * DH + 8]))
            gT_sc[c] = g
            g_sc[c] = jnp.concatenate([1.0 - g] * 16, axis=0).T

        kv_at = ((5, 0), (5, 4), (6, 0), (6, 4))
        x_op = _operands(LHS, lambda r, k: x_sc[r * TQ:(r + 1) * TQ, k * DQ:(k + 1) * DQ])
        w_op = _operands(RHS, lambda k, j: wq_sc[k * DQ:(k + 1) * DQ, j * DQ:(j + 1) * DQ])

        def operands(step, r1, r2):
            for copy in copies.get(step, ()):
                copy.wait()
            if step in kv_at:
                kv_gate(kv_at.index(step))
            rhs, lhs = w_op(r1, r2), x_op(r1, r2)
            xop_sc[7 * r1 + r2] = pltpu.bitcast(lhs, u32)
            return lhs, rhs

        def emit(r, j, val):
            qT_sc[r, j * DQ:(j + 1) * DQ, :] = (val * Q_SCALE).astype(bf16).T

        _strassen2(PROJ_ORDER, operands, emit)

    def attend(slot, h_pv, h_qk, l_sc, oT_sc=None, qf_sc=None):
        assist = h_pv is not None and h_qk is not None
        regs = [KC // 16 - (assist and (c in VC or c in FC)) for c in range(NC)]
        places = [(c, u) for c in range(NC) for u in range(regs[c])][8:]
        pieces = [(g, t) for g in range(2 * NV) for t in LANES] if assist else []
        piece_at = {places[(a + 1) * len(places) // len(pieces) - 1]: piece for a, piece in enumerate(pieces)}
        for qb in range(NQ):
            probs = p_sc[qb].at[_ds(slot * (S // 2), S // 2, S // 2)]

            def put(row, p):
                probs[row:row + p.shape[0] // 2] = pltpu.bitcast(p.astype(bf16), u32)

            extra = _Memo(lambda g, t: _vpu_scores(kv_sc, qf_sc.at[slot, qb], g, t))
            sums = []
            for c in range(NC):
                row = c * KC // 2
                if h_pv is not None:
                    p = probs[row:row + KC // 2]
                if h_qk is not None:
                    keys = []
                    for u in range(regs[c]):
                        k = k_sc[row + 8 * u:row + 8 * (u + 1), :]
                        if (c, u) in piece_at:
                            k = _tie(h_qk < 0, extra[piece_at[c, u]], k)
                        keys.append(k)
                    e = jnp.exp2(_dot(pltpu.bitcast(jnp.concatenate(keys, axis=0), bf16), q_rows(qb, h_qk)))
                    part = _tree_sum([e[8 * j:8 * (j + 1)] for j in range(2 * regs[c])])
                    den = part if c == 0 else den + part
                    put(row, e)
                    if assist and c in FC:
                        e = jnp.exp2(sf_sc[qb, h_qk - HU, 16 * c:16 * (c + 1)])
                        den = den + (e[:8] + e[8:])
                        put(row + KC // 2 - 8, e)
                if h_pv is not None:
                    vT = vT_sc[c * KC // TQ, :, c * KC % TQ:c * KC % TQ + KC]
                    part = _dot(pltpu.bitcast(vT, bf16), pltpu.bitcast(p, bf16))
                    num = part if c == 0 else num + part
            if assist:
                for i, c in enumerate(VC):
                    e = jnp.exp2(jnp.concatenate(
                        [jnp.concatenate([extra[g, t] for t in LANES], axis=1) for g in (2 * i, 2 * i + 1)], axis=0))
                    put((c + 1) * KC // 2 - 8, e)
                    sums.append(e[:8] + e[8:])
                qf_sc[slot, qb] = q_rows(qb, jnp.minimum(h_qk + HU, H - 1)).astype(f32)
            if h_qk is not None:
                den = jnp.sum(_tree_sum([den] + sums), axis=0, keepdims=True)
                l_sc[qb, h_qk // HG, pl.ds(h_qk % HG, 1), :] = den
            if h_pv is not None:
                oT_sc[_ds(qb * D + h_pv * DH, DH, DH), :] = num

    def gate_up(l_sc, g_sc, xop_sc, w_sc, kf_sc, qf_sc):
        def w_copies(j):
            return [pltpu.make_async_copy(src.at[:, _ds(j * 512, 512, 512)], w_sc[i].at[j % 2], wsems.at[i, j % 2])
                    for i, src in enumerate((wg_hbm, wu_hbm))]

        def unit(j, u):
            at = jnp.minimum(j * NU + u, (H - HU) * NQ - 1)
            return at % NQ, at // NQ

        def stage_queries(j):
            for u in range(NU):
                qb, h = unit(j, u)
                qf_sc[u] = q_rows(qb, h + HU).astype(f32)

        for copy in w_copies(0):
            copy.start()

        def first_heads(slot, carry):
            for ref, steps in ((kf_sc, FC), (kv_sc, VC)):
                for i, c in enumerate(steps):
                    stop = (c + 1) * KC // 2
                    k = pltpu.bitcast(k_sc[stop - 8:stop, :], bf16).astype(f32)
                    k = jnp.where(slot == 0, k[:8], k[8:])
                    for d in range(DH):
                        ref[2 * i + slot, d] = jnp.broadcast_to(k[:, d:d + 1], (8, 128))
            stage_queries(0)
            attend(slot, None, slot, l_sc)
            return carry

        lax.fori_loop(0, HU, first_heads, 0)

        pieces = [(u, g, t) for u in range(NU) for g in range(2 * NF) for t in LANES]
        share = np.cumsum(np.repeat(FFN_SHARE, TQ // 16))
        done_by = np.concatenate([[0], share * len(pieces) // share[-1]])

        def body(j, carry):
            for copy in w_copies(j):
                copy.wait()

            @pl.when(j + 1 < NG)
            def _():
                for copy in w_copies(j + 1):
                    copy.start()

            wide = _Memo(lambda k, n: [w[j % 2, k * DQ:(k + 1) * DQ, n * 256:(n + 1) * 256].astype(f32) for w in w_sc])
            w_op = _operands(RHS, lambda k, n: jnp.concatenate(
                [w[:, n % 2 * 128:(n % 2 + 1) * 128] for w in wide[k, n // 2]], axis=1))

            def operands(step, r1, r2):
                rhs = w_op(r1, r2)
                first = (7 * step[0] + step[1]) * (TQ // 16)
                rows = []
                for a in range(TQ // 16):
                    x = xop_sc[7 * r1 + r2, 8 * a:8 * (a + 1)]
                    for u, g, t in pieces[done_by[first + a]:done_by[first + a + 1]]:
                        val = _vpu_scores(kf_sc, qf_sc.at[u], g, t)
                        qb, h = unit(j, u)
                        sf_sc[qb, h, 8 * g:8 * (g + 1), 128 * t:128 * (t + 1)] = val
                        x = jnp.concatenate([_tie(j < 0, val, x[:, :128]), x[:, 128:]], axis=1)
                    rows.append(x)
                return pltpu.bitcast(jnp.concatenate(rows, axis=0), bf16), rhs

            hidden, stored = {}, []
            mids = _Memo(lambda r1, i: _lin(LHS[r1], lambda o: hidden[_rc(o, i)]))

            def emit(r, n, val):
                hidden[r, 3 - n] = jnp.maximum(val[:, :128], 0.0) * val[:, 128:] * g_sc[r]
                for r1 in range(7):
                    for pair, part in ((0, 0), (1, 0), (0, 1), (1, 1)):
                        ready = all(_rc(o, 2 * pair + k) in hidden for o, _ in LHS[r1] for k in range(part + 1))
                        if ready and (r1, pair, part) not in stored:
                            stored.append((r1, pair, part))
                            for half in range(2):
                                i, rows = (2 * pair + half + ROT[r1]) % 4, slice(half * RB, (half + 1) * RB)
                                a = mids[r1, 2 * pair][rows]
                                h_sc[r1, part, i, j] = T4[i] * a + mids[r1, 2 * pair + 1][rows] if part else a

            _strassen2(FFN_ORDER, operands, emit)
            stage_queries(j + 1)
            return carry

        lax.fori_loop(0, NG, body, 0)

    def attention(l0_sc, l_sc, oT_sc, wo_sc, wd_sc, qf_sc):
        def finish(qb, grp):
            w = gT_sc[qb, 0:1, :] / l_sc[qb, grp, :HG]
            tile = oT_sc.at[_ds(qb * D + grp * 128, 128, 128)]
            o = jnp.concatenate([tile[t * DH:(t + 1) * DH, :] * w[t:t + 1] for t in range(HG)], axis=0)
            for b in range(0, TQ, 128):
                tile[:, b:b + 128] = o[:, b:b + 128].T

        late = [pltpu.make_async_copy(wd_hbm, wd_sc, sems.at[11]), pltpu.make_async_copy(wo_hbm, wo_sc, sems.at[12])]
        for copy in late:
            copy.start()
        l_sc[NQ - 1, H // HG] = jnp.ones(l_sc.shape[2:], f32)
        oT_sc[NQ * D:] = jnp.zeros((128, TQ), f32)
        for qb in range(NQ):
            l_sc[qb, 0, :HU] = l0_sc[qb, 0, :HU]
            for slot in range(HU):
                qf_sc[slot, qb] = q_rows(qb, HU + slot).astype(f32)

        def body(i, carry):
            for slot in range(HU):
                u = (i - 1) * HU - HG + slot
                finish(jnp.where(u < 0, NQ - 1, u % NQ), jnp.where(u < 0, H // HG, u // NQ))
            for slot in range(HU):
                attend(slot, (i - 1) * HU + slot, i * HU + slot, l_sc, oT_sc, qf_sc)
            return carry

        lax.fori_loop(1, H // HU, body, 0)
        for copy in late:
            copy.wait()
        for u in range(H - HU - HG, H - NQ):
            finish(u % NQ, u // NQ)
        for slot in range(HU):
            attend(slot, H - HU + slot, None, l_sc, oT_sc)
        for qb in range(NQ):
            finish(qb, H // HG - 1)

        def within(x, big):
            return jnp.where((x >= 2.0 ** -big) & (x <= 2.0 ** big), 1.0, 0.0)

        ok = None
        for qb in range(NQ):
            for grp in range(H // HG):
                part = within(l_sc[qb, grp, :HG], 60)
                ok = part if ok is None else jnp.minimum(ok, part)
        v_abs = jnp.abs(jnp.concatenate([pltpu.bitcast(vT_sc[c], bf16) for c in range(NQ)], axis=0).astype(f32))
        v_top = jnp.max(jnp.max(v_abs, axis=0, keepdims=True), axis=1, keepdims=True)
        safe = jnp.min(jnp.minimum(ok, within(v_top, 30))) > 0.5

        @pl.when(jnp.logical_not(safe))
        def _():
            @pl.loop(0, H * NQ)
            def _(u):
                qb, h = u % NQ, u // NQ
                s = _dot(pltpu.bitcast(k_sc[...], bf16), q_rows(qb, h))
                p = jnp.exp2(s - jnp.max(s, axis=0, keepdims=True))
                vT = jnp.concatenate([pltpu.bitcast(vT_sc[c], bf16) for c in range(NQ)], axis=1)
                l_sc[qb, h // HG, pl.ds(h % HG, 1), :] = jnp.sum(p, axis=0, keepdims=True)
                oT_sc[_ds(qb * D + h * DH, DH, DH), :] = _dot(vT, p.astype(bf16))

            @pl.loop(0, H // HG * NQ)
            def _(u):
                finish(u % NQ, u // NQ)

    def down(o_sc, wo_sc, wd_sc):
        out_sc = qT_sc

        def pick(table, n):
            vals = []
            for col in zip(*table):
                v = col[0]
                for r in range(1, len(col)):
                    if col[r] != col[r - 1]:
                        v = jnp.where(n >= r, col[r], v)
                vals.append(v)
            return vals

        def two(terms):
            coef = float(terms[1][1]) if len(terms) > 1 else 0.0
            return divmod(terms[0][0], 2) + divmod(terms[-1][0], 2) + (coef,)

        steps = []
        for n, r in enumerate(DOWN_OUTER):
            full = [o for o, terms in enumerate(OUT)
                    if r in dict(terms) and all(t in DOWN_OUTER[:n + 1] for t, _ in terms)]
            assert len(full) == (n >= 3) and (not full or dict(OUT[full[0]])[r] == 1)
            others = [(DOWN_OUTER.index(t), float(sign)) for t, sign in OUT[full[0]] if t != r] if full else []
            others += [(0, 0.0)] * (3 - len(others))
            steps.append((r, ROT[r], full[0] if full else 0) + sum(others, ()))

        def body(n, carry):
            *a_blk, a_coef = pick([two(LHS[r]) for r in DOWN_OUTER], n)
            *b_blk, b_coef = pick([two(RHS[r]) for r in DOWN_OUTER], n)
            r1, rot, blk, i0, k0, i1, k1, i2, k2 = pick(steps, n)
            home = [(i + 4 - rot) & 3 for i in range(4)]

            def o_blk(row, col, i, half, u):
                ref = o_sc.at[_ds((2 * row + (home[i] >> 1)) * D + (2 * col + half) * DQ, DQ, DQ),
                              _ds((home[i] & 1) * RB, RB, RB)]
                return jnp.concatenate([ref[u * 128:(u + 1) * 128, b:b + 128] for b in range(0, RB, 128)], axis=0)

            def w_blk(row, col, half, j, t):
                cols = _ds(col * 512, 512, 512)
                if t < NG:
                    ref, top = wd_sc.at[_ds((1 - row) * 256, F - 256, 256), cols], t * 512 + (1 - half) * 128
                else:
                    ref, top = wo_sc.at[_ds(row * 512, 512, 512), cols], half * DQ + (t - NG) * 128
                return ref[top:top + 128, j * 128:(j + 1) * 128].astype(f32)

            def scaled(coef, v):
                return v if coef == 1 else coef * v

            o_mid = _Memo(lambda *at: o_blk(*a_blk[:2], *at) + a_coef * o_blk(*a_blk[2:], *at))
            w_mid = _Memo(lambda *at: w_blk(*b_blk[:2], *at) + b_coef * w_blk(*b_blk[2:], *at))
            h_ref = h_sc.at[r1]
            a = _Memo(lambda i, t: h_ref[0, i, t] if t < NG else o_mid[i, 0, t - NG])
            b = _Memo(lambda i, t: h_ref[1, i, t] if t < NG else T4[i] * o_mid[i, 0, t - NG] + o_mid[i, 1, t - NG])
            c = _Memo(lambda j, t: w_mid[0, j, t] - T4[j] * w_mid[1, j, t])
            r = _Memo(lambda i, j, t: scaled(1 / (T4[j] - T4[i]), b[i, t] - b[j, t]))
            s = _Memo(lambda i, j, t: c[i, t] + c[j, t])

            def product(lhs, rhs):
                parts = []
                for tiles in (range(0, 5), range(5, NG + 2)):
                    w = jnp.concatenate([rhs(t) for t in tiles], axis=0).astype(bf16)
                    parts.append(_dot(jnp.concatenate([lhs(t) for t in tiles], axis=1).astype(bf16), w))
                return parts[0] + parts[1]

            def emit(i, j, val):
                staged = out_sc.at[blk, _ds(home[i] * RB, RB, RB)]

                def kept(step):
                    return p_sc[j].at[_ds((home[i] * 7 + step) * (RB // 4), RB // 4, RB // 4)]

                for t in range(0, RB, 64):
                    rows = slice(t // 4, t // 4 + 16)
                    new = jnp.concatenate([val[z:z + 16] for z in range(t, t + 64, 16)], axis=1)
                    old = [pltpu.bitcast(kept(step)[rows], f32) for step in (i0, i1, i2)]
                    total = jnp.where(n > 0, k0 * old[0] + k1 * old[1] + k2 * old[2], 0.0) + new
                    kept(n)[rows] = pltpu.bitcast(new, u32)
                    total = jnp.concatenate([total[:, z:z + 128] for z in range(0, TQ, 128)], axis=0)
                    staged[t:t + 64, j * 128:(j + 1) * 128] = total.astype(bf16)

                @pl.when(n >= 3)
                def _():
                    dst = o_hbm.at[_ds((4 * (blk >> 1) + home[i]) * RB, RB, RB),
                                   _ds((blk & 1) * 512 + j * 128, 128, 128)]
                    pltpu.make_async_copy(staged.at[:, j * 128:(j + 1) * 128], dst, osem).start()

            prods, emitted = {}, []
            for name in DOWN_INNER.split():
                i, j = int(name[1]), int(name[-1])
                lo, hi = min(i, j), max(i, j)
                if name[0] == "P":
                    prods[name] = product(lambda t: a[i, t], lambda t: c[i, t])
                elif name[0] == "Q":
                    prods[name] = product(lambda t: b[i, t], lambda t: w_mid[1, i, t])
                elif name[0] == "R":
                    prods[name] = product(lambda t: r[lo, hi, t], lambda t: s[lo, hi, t])
                else:
                    op = jnp.add if i < j else jnp.subtract
                    prods[name] = product(lambda t: a[i, t] + r[lo, hi, t],
                                          lambda t: op(s[lo, hi, t], scaled(T4[hi] - T4[lo], w_mid[1, j, t])))
                for i in range(4):
                    for j in range(4):
                        need = [f"P{i}", f"Q{j}"] + ([f"R{min(i, j)}{max(i, j)}", f"S{i}{j}"] if i != j else [])
                        if (i, j) not in emitted and all(x in prods for x in need):
                            emitted.append((i, j))
                            v = [prods[x] for x in need]
                            emit(i, j, v[0] + v[1] if i == j else v[3] + (v[1] - v[0] - v[2]))
            return carry

        lax.fori_loop(0, 7, body, 0)
        pltpu.make_async_copy(o_hbm, o_hbm, osem).wait()

    def run(l0_sc):
        def front(g_sc, xop_sc):
            pl.run_scoped(lambda *refs: project(g_sc, xop_sc, *refs),
                          V((S, D), bf16), V((D, D), bf16), V((2, DH, D), bf16), V((64, 128), bf16))
            pl.run_scoped(lambda *refs: gate_up(l0_sc, g_sc, xop_sc, *refs),
                          [V((2, D, 512), bf16)] * 2, V((2 * NF, DH, 8, 128), f32), V((NU, DH, TQ), f32))

        def back(l_sc, oT_sc, wo_sc, wd_sc, qf_sc):
            attention(l0_sc, l_sc, oT_sc, wo_sc, wd_sc, qf_sc)
            down(oT_sc, wo_sc, wd_sc)

        pl.run_scoped(front, V((NQ, TQ, 128), f32), V((49, TQ // 2, DQ), u32))
        pl.run_scoped(back, V((NQ, H // HG + 1, 8, TQ), f32), V((NQ * D + 128, TQ), f32),
                      V((D, D), bf16), V((F, D), bf16), V((HU, NQ, DH, TQ), f32))

    pl.run_scoped(run, V((NQ, 1, 8, TQ), f32))


@jax.jit
def pallas_gated_mix__grouped_kv_mqa__glu_gated_reglu__prompt_kernel(
    A_x: jax.Array,
    A_wq: jax.Array,
    A_wk: jax.Array,
    A_wv: jax.Array,
    A_wo: jax.Array,
    B_x: jax.Array,
    B_W_gate: jax.Array,
    B_W_up: jax.Array,
    B_W_down: jax.Array,
    gate_w: jax.Array,
):
    del B_x
    assert A_x.shape == (1, S, D) and B_W_gate.shape == (D, F) and A_wk.shape == (D, DH)
    hbm, V = pl.BlockSpec(memory_space=pl.ANY), pltpu.VMEM
    out = pl.pallas_call(
        _kernel,
        in_specs=[hbm] * 9,
        out_specs=hbm,
        out_shape=jax.ShapeDtypeStruct((S, D), bf16),
        scratch_shapes=[
            V((S // 2, DH), u32),
            V((NQ, DH // 2, TQ), u32),
            V((NQ, D, TQ), bf16),
            V((NQ, 8, TQ), f32),
            V((7, 2, 4, NG, RB, 128), f32),
            [V((S, TQ), u32)] * NQ,
            V((2 * NV, DH, 8, 128), f32),
            V((NQ, H - HU, 16 * NF, TQ), f32),
            pltpu.SemaphoreType.DMA((13,)),
            pltpu.SemaphoreType.DMA((2, 2)),
            pltpu.SemaphoreType.DMA,
        ],
        compiler_params=pltpu.CompilerParams(vmem_limit_bytes=128 * 1024 * 1024),
        name="gated_mix_kernel",
    )(A_x.reshape(S, D), A_wq, A_wk.T, A_wv.T, A_wo, B_W_gate, B_W_up, B_W_down, gate_w.reshape(D // 128, 128))
    return out.reshape(A_x.shape)
```
